```python
import os as _os
_os.environ.setdefault('JAX_PLATFORMS', 'cpu')
import jax
import jax.numpy as jnp

def _softmax(x, axis=-1):
    return jax.nn.softmax(x, axis=axis)

def _gelu(x):
    return jax.nn.gelu(x, approximate=True)

def _silu(x):
    return jax.nn.silu(x)

def _sigmoid(x):
    return jax.nn.sigmoid(x)

def _layernorm(x, axis=-1, eps=1e-05):
    m = jnp.mean(x, axis=axis, keepdims=True)
    v = jnp.var(x, axis=axis, keepdims=True)
    return (x - m) / jnp.sqrt(v + eps)

def _scatter_add(tgt, idx, src, axis=0):
    return tgt.at[idx].add(src)

def _segment_sum(src, seg, n):
    return jax.ops.segment_sum(src, seg, n)

class _Rng:

    def __init__(self, key):
        self._k = key

    def _next(self):
        self._k, sub = jax.random.split(self._k)
        return sub

    def normal(self, shape):
        return jax.random.normal(self._next(), shape, dtype=jnp.bfloat16)

    def randint(self, lo, hi, shape):
        return jax.random.randint(self._next(), shape, lo, hi, dtype=jnp.int32)

    def uniform(self, shape, lo=0.0, hi=1.0):
        return jax.random.uniform(self._next(), shape, jnp.bfloat16, lo, hi)

    def permutation(self, n):
        return jax.random.permutation(self._next(), n)
kernel_name = 'parallel_sum__memory_aug_recurrent_mem_tr__dense_activation_gelu__prompt'

def setup_inputs():
    _rng = _Rng(jax.random.key(int.from_bytes(__import__("os").urandom(4), "little")))
    _w = lambda a: (lambda t: t.astype(jnp.bfloat16) if jnp.issubdtype(t.dtype, jnp.floating) else t)(jnp.asarray(a))

    def _A_setup():
        B, S, Dm = (1, 2048, 1024)
        H, Dh = (32, 128)
        M, seg = (8, 32)
        seg = min(seg, S)
        S = S // seg * seg
        return {'x': _w((lambda *s: _rng.normal(s) * 0.05)(B, S, Dm)), 'mem0': _w((lambda *s: _rng.normal(s) * 0.2)(B, M, Dm)), 'Wq': _w((lambda *s: _rng.normal(s) * 0.8)(Dm, H, Dh) * Dm ** (-0.5)), 'Wk': _w((lambda *s: _rng.normal(s) * 0.8)(Dm, H, Dh) * Dm ** (-0.5)), 'Wv': _w((lambda *s: _rng.normal(s) * 0.2)(Dm, H, Dh) * Dm ** (-0.5)), 'Wo': _w((lambda *s: _rng.normal(s) * 0.2)(H, Dh, Dm) * (H * Dh) ** (-0.5)), 'seg_len': seg}
    _A_in = _A_setup()

    def _B_setup():
        B, S, D, F = (1, 2048, 1024, 3584)
        return {'x': _w((lambda *s: _rng.normal(s) * 0.05)(B, S, D)), 'w1': _w((lambda *s: _rng.normal(s) * 0.1)(D, F) * D ** (-0.5)), 'b1': _w((lambda *s: _rng.normal(s) * 0.1)(F) * 0.01), 'w2': _w((lambda *s: _rng.normal(s) * 0.1)(F, D) * F ** (-0.5)), 'b2': _w((lambda *s: _rng.normal(s) * 0.05)(D) * 0.01)}
    _B_in = _B_setup()
    return {'A_x': _A_in['x'], 'A_mem0': _A_in['mem0'], 'A_Wq': _A_in['Wq'], 'A_Wk': _A_in['Wk'], 'A_Wv': _A_in['Wv'], 'A_Wo': _A_in['Wo'], 'A_seg_len': _A_in['seg_len'], 'B_x': _B_in['x'], 'B_w1': _B_in['w1'], 'B_b1': _B_in['b1'], 'B_w2': _B_in['w2'], 'B_b2': _B_in['b2']}

def reference(A_x, A_mem0, A_Wq, A_Wk, A_Wv, A_Wo, A_seg_len, B_x, B_w1, B_b1, B_w2, B_b2):

    def _A_ref(x, mem0, Wq, Wk, Wv, Wo, seg_len):
        B, S, Dm = x.shape
        H, Dh = (Wq.shape[1], Wq.shape[2])
        M = mem0.shape[1]
        scale = Dh ** (-0.5)
        n_seg = S // seg_len
        L = M + seg_len
        idx = jnp.arange(L)
        mask = (idx[:, None] < M) | (idx[:, None] >= idx[None, :])
        mem = mem0
        outs = []
        for s in range(n_seg):
            xs = x[:, s * seg_len:(s + 1) * seg_len, :].copy()
            h = jnp.concatenate([mem, xs], axis=1)
            q = jnp.einsum('btd,dhe->bhte', h, Wq)
            k = jnp.einsum('btd,dhe->bhte', h, Wk)
            v = jnp.einsum('btd,dhe->bhte', h, Wv)
            scores = jnp.einsum('bhqe,bhke->bhqk', q, k) * scale
            scores = jnp.where(mask[None, None], scores, -1000000000.0)
            p = _softmax(scores, axis=-1)
            o = jnp.einsum('bhqk,bhke->bhqe', p, v)
            o = jnp.einsum('bhte,hed->btd', o, Wo)
            mem = o[:, :M, :].copy()
            outs.append(o[:, M:, :])
        return jnp.concatenate(outs, axis=1)

    def _B_ref(x, w1, b1, w2, b2):
        h = jnp.einsum('bsd,df->bsf', x, w1) + b1
        h = _gelu(h)
        return jnp.einsum('bsf,fd->bsd', h, w2) + b2
    x = A_x
    xn = _layernorm(x, axis=-1)
    return x + _A_ref(xn, A_mem0, A_Wq, A_Wk, A_Wv, A_Wo, A_seg_len) + _B_ref(xn, B_w1, B_b1, B_w2, B_b2)
```

```python
import functools

import jax
import jax.numpy as jnp
from jax import lax
from jax.experimental import pallas as pl
from jax.experimental.pallas import tpu as pltpu

F32 = jnp.float32
BF16 = jnp.bfloat16
U32 = jnp.uint32

BCH = 512
AG = 32
LOG2E = 1.4426950408889634


def _dot(a, b):
    return jnp.dot(a, b, preferred_element_type=F32)


def _bf(u):
    return pltpu.bitcast(u, BF16)


def _u32(v):
    return pltpu.bitcast(v, U32)


def _kernel(mem0_ref, b1_ref, b2_ref,
            x_hbm, wq_hbm, wk_hbm, wv_hbm, wo_hbm, w1_hbm, w2_hbm,
            o_hbm,
            wq_s, wk_s, wv_s, wo_s, w1_s, w2_s, x_s, xn_s, xa_s, xb_s, bm_s,
            st_q, st_k, st_v, st_o, st_w1, st_w2, st_out,
            xsems, wsems, asems, osems,
            *, S, Dm, H, Dh, M, SEG, FF):
    NP = S // (2 * SEG)
    L = M + SEG
    PR = 2 * SEG
    c_exp = (Dh ** (-0.5)) * LOG2E
    HD = H * Dh
    HP = H // 2
    NBC = FF // BCH
    XB = NBC + 1
    XR = S // XB
    PPB = XR // PR
    NCH = 16
    DCH = Dm // NCH
    QROWS = DCH * H
    OROWS = HD // NCH
    R1 = (S - XR) // NCH

    def x_dma(b):
        return pltpu.make_async_copy(
            x_hbm.at[pl.ds(pl.multiple_of(b * XR, XR), XR), :],
            x_s.at[pl.ds(pl.multiple_of(b * XR, XR), XR), :], xsems.at[b % 2])

    def w_dmas(c, slot):
        off = pl.multiple_of(c * BCH, BCH)
        return (
            pltpu.make_async_copy(w1_hbm.at[:, pl.ds(off, BCH)], st_w1.at[slot],
                                  wsems.at[0, slot]),
            pltpu.make_async_copy(w2_hbm.at[pl.ds(off, BCH), :], st_w2.at[slot],
                                  wsems.at[1, slot]),
        )

    def a_dmas(c, slot):
        rq = pl.ds(pl.multiple_of(c * QROWS, QROWS), QROWS)
        ro = pl.ds(pl.multiple_of(c * OROWS, OROWS), OROWS)
        return (
            pltpu.make_async_copy(wq_hbm.at[rq, :], st_q.at[slot], asems.at[0, slot]),
            pltpu.make_async_copy(wk_hbm.at[rq, :], st_k.at[slot], asems.at[1, slot]),
            pltpu.make_async_copy(wv_hbm.at[rq, :], st_v.at[slot], asems.at[2, slot]),
            pltpu.make_async_copy(wo_hbm.at[ro, :], st_o.at[slot], asems.at[3, slot]),
        )

    x_dma(0).start()
    for d in w_dmas(0, 0):
        d.start()
    x_dma(1).start()

    def ln_pair(j):
        r = pl.multiple_of(j * PR, PR)
        xb = x_s[pl.ds(r, PR), :].astype(F32)
        mu = jnp.mean(xb, axis=-1, keepdims=True)
        xc = xb - mu
        var = jnp.mean(xc * xc, axis=-1, keepdims=True)
        xn = xc / jnp.sqrt(var + 1e-05)
        xn_s[pl.ds(pl.multiple_of(j * SEG, SEG), SEG), :] = _u32(xn.astype(BF16))
        z = jnp.zeros((M, Dm), F32)
        xa_s[j] = _u32(jnp.concatenate([z, xn[0:SEG + M]], axis=0).astype(BF16))
        xb_s[j] = _u32(jnp.concatenate([z, xn[SEG + M:PR]], axis=0).astype(BF16))

    def ln_block(b):
        def body(i, carry):
            ln_pair(b * PPB + i)
            return carry
        lax.fori_loop(0, PPB, body, 0)

    x_dma(0).wait()
    ln_block(0)
    bm_s[pl.ds(0, XR), :] = jnp.broadcast_to(b2_ref[...].astype(F32), (XR, Dm))

    def phase0_body(c, carry):
        slot = c % 2
        off = pl.multiple_of(c * BCH, BCH)

        @pl.when(c + 1 < NBC)
        def _():
            for d in w_dmas(c + 1, 1 - slot):
                d.start()

        @pl.when(c + 2 < XB)
        def _():
            x_dma(c + 2).start()

        @pl.when(c + 1 == NBC)
        def _():
            for d in a_dmas(0, 0):
                d.start()

        for d in w_dmas(c, slot):
            d.wait()
        w1_s[:, pl.ds(off, BCH)] = _u32(st_w1[slot])
        w2_s[pl.ds(pl.multiple_of(c * (BCH // 2), BCH // 2), BCH // 2), :] = _u32(st_w2[slot])

        xs = _bf(xn_s[pl.ds(0, XR // 2), :])
        hb = _dot(xs, _bf(w1_s[:, pl.ds(off, BCH)])) + b1_ref[:, pl.ds(off, BCH)].astype(F32)
        hb = jax.nn.gelu(hb, approximate=True).astype(BF16)
        bm_s[pl.ds(0, XR), :] += _dot(
            hb, _bf(w2_s[pl.ds(pl.multiple_of(c * (BCH // 2), BCH // 2), BCH // 2), :]))

        x_dma(c + 1).wait()
        ln_block(c + 1)
        return carry

    lax.fori_loop(0, NBC, phase0_body, 0)

    def qkv_repack(stage_ref, slot, ws_ref, c):
        u = _u32(stage_ref[slot]).reshape(DCH // 2, 2, HP, Dh)
        ev = u[:, 0]
        od = u[:, 1]
        lo = (ev & jnp.uint32(0xFFFF)) | (od << 16)
        hi = (ev >> 16) | (od & jnp.uint32(0xFFFF0000))
        lo = jnp.swapaxes(lo, 0, 1)
        hi = jnp.swapaxes(hi, 0, 1)
        p0 = pl.multiple_of(c * (DCH // 2), DCH // 2)
        for j in range(HP):
            ws_ref[pl.ds(p0, DCH // 2), pl.ds((2 * j) * Dh, Dh)] = lo[j]
            ws_ref[pl.ds(p0, DCH // 2), pl.ds((2 * j + 1) * Dh, Dh)] = hi[j]

    def phase1_body(c, carry):
        slot = c % 2

        @pl.when(c + 1 < NCH)
        def _():
            for d in a_dmas(c + 1, 1 - slot):
                d.start()

        def first():
            for d in a_dmas(c, slot):
                d.wait()
            qkv_repack(st_q, slot, wq_s, c)

        def wo_copy():
            ro = pl.multiple_of(c * (OROWS // 2), OROWS // 2)
            wo_s[pl.ds(ro, OROWS // 2), :] = _u32(st_o[slot])

        side = [None, first,
                lambda: qkv_repack(st_k, slot, wk_s, c),
                lambda: qkv_repack(st_v, slot, wv_s, c),
                wo_copy]

        r0 = pl.multiple_of(XR + c * R1, 16)
        xs = _bf(xn_s[pl.ds(pl.multiple_of(r0 // 2, 8), R1 // 2), :])
        acc = None
        for hc in range(NBC):
            cs = pl.ds(hc * BCH, BCH)
            hb = _dot(xs, _bf(w1_s[:, cs])) + b1_ref[:, cs].astype(F32)
            hb = jax.nn.gelu(hb, approximate=True).astype(BF16)
            part = _dot(hb, _bf(w2_s[pl.ds(hc * (BCH // 2), BCH // 2), :]))
            acc = part if acc is None else acc + part
            if hc < len(side) and side[hc] is not None:
                side[hc]()
        bm_s[pl.ds(r0, R1), :] = acc + b2_ref[...].astype(F32)
        return carry

    lax.fori_loop(0, NCH, phase1_body, 0)

    qi = lax.broadcasted_iota(jnp.int32, (L, L), 0)
    ki = lax.broadcasted_iota(jnp.int32, (L, L), 1)

    def out_dma(j):
        return pltpu.make_async_copy(
            st_out.at[j % 2], o_hbm.at[pl.ds(pl.multiple_of(j * PR, PR), PR), :],
            osems.at[j % 2])

    def pair_body(j, mem_u):
        mask = (qi < M) | (qi >= ki)
        wq = _bf(wq_s[...])
        wk = _bf(wk_s[...])
        wv = _bf(wv_s[...])

        def attn(q, k, v):
            outs = []
            for g0 in range(0, H, AG):
                hs = range(g0, g0 + AG)
                us = [lax.dot_general(q[:, hh * Dh:(hh + 1) * Dh], k[:, hh * Dh:(hh + 1) * Dh],
                                      (((1,), (1,)), ((), ())),
                                      preferred_element_type=F32) for hh in hs]
                ps = []
                for u in us:
                    u = jnp.where(mask, u * c_exp, -1000000000.0)
                    mx = jnp.max(u, axis=-1, keepdims=True)
                    e = jnp.exp2(u - mx)
                    l = jnp.sum(e, axis=-1, keepdims=True)
                    r = pl.reciprocal(l, approx=True)
                    r = r * (2.0 - l * r)
                    ps.append((e * r).astype(BF16))
                for hh, p in zip(hs, ps):
                    outs.append(_dot(p, v[:, hh * Dh:(hh + 1) * Dh]))
            return outs

        xa_s[j, pl.ds(0, M // 2), :] = mem_u
        lhs_a = _bf(xa_s[j])
        qa, ka, va = _dot(lhs_a, wq), _dot(lhs_a, wk), _dot(lhs_a, wv)
        oa = attn(qa[0:L].astype(BF16), ka[0:L].astype(BF16), va[0:L].astype(BF16))
        ya = _dot(jnp.concatenate([o[0:L - M].astype(BF16) for o in oa], axis=1),
                  _bf(wo_s[...]))

        xb_s[j, pl.ds(0, M // 2), :] = _u32(ya[0:M].astype(BF16))
        lhs_b = _bf(xb_s[j])
        qb, kb, vb = _dot(lhs_b, wq), _dot(lhs_b, wk), _dot(lhs_b, wv)

        def asm(tb, ta):
            return jnp.concatenate([tb[0:M], ta[L:L + M], tb[M:SEG]], axis=0).astype(BF16)

        ob = attn(asm(qb, qa), asm(kb, ka), asm(vb, va))
        yb = _dot(jnp.concatenate(
            [jnp.concatenate([o, oa_[L - M:L]], axis=0).astype(BF16) for o, oa_ in zip(ob, oa)],
            axis=1), _bf(wo_s[...]))

        r = pl.multiple_of(j * PR, PR)
        a_part = jnp.concatenate([ya[M:L - M], yb[L:L + M], yb[M:L]], axis=0)
        xr = x_s[pl.ds(r, PR), :].astype(F32)
        bo = bm_s[pl.ds(r, PR), :]

        @pl.when(j >= 2)
        def _():
            out_dma(j - 2).wait()

        st_out[j % 2] = (xr + a_part.astype(BF16).astype(F32)
                         + bo.astype(BF16).astype(F32)).astype(BF16)
        out_dma(j).start()
        return _u32(yb[0:M].astype(BF16))

    ntrips = NP
    lax.fori_loop(0, ntrips, pair_body, _u32(mem0_ref[...]))
    if ntrips >= 2:
        out_dma(ntrips - 2).wait()
    if ntrips >= 1:
        out_dma(ntrips - 1).wait()


@functools.partial(jax.jit, static_argnames=("A_seg_len",))
def pallas_parallel_sum__memory_aug_recurrent_mem_tr__dense_activation_gelu__prompt_kernel(
        A_x, A_mem0, A_Wq, A_Wk, A_Wv, A_Wo, A_seg_len, B_x, B_w1, B_b1, B_w2, B_b2):
    Bb, S, Dm = A_x.shape
    assert Bb == 1
    _, M, _ = A_mem0.shape
    _, H, Dh = A_Wq.shape
    FF = B_w1.shape[1]
    SEG = int(A_seg_len)
    HD = H * Dh
    NP = S // (2 * SEG)
    XR = S // (FF // BCH + 1)

    x2 = A_x.reshape(S, Dm)
    mem2 = A_mem0.reshape(M, Dm)
    wq2 = A_Wq.reshape(Dm * H, Dh)
    wk2 = A_Wk.reshape(Dm * H, Dh)
    wv2 = A_Wv.reshape(Dm * H, Dh)
    wo2 = A_Wo.reshape(HD, Dm)
    b1r = B_b1.reshape(1, FF)
    b2r = B_b2.reshape(1, Dm)
    QR = Dm // 16 * H

    vmem = pl.BlockSpec(memory_space=pltpu.VMEM)
    anyspec = pl.BlockSpec(memory_space=pl.ANY)
    kern = functools.partial(_kernel, S=S, Dm=Dm, H=H, Dh=Dh, M=M, SEG=SEG, FF=FF)
    out = pl.pallas_call(
        kern,
        out_shape=jax.ShapeDtypeStruct((S, Dm), A_x.dtype),
        in_specs=[vmem, vmem, vmem] + [anyspec] * 7,
        out_specs=anyspec,
        scratch_shapes=[
            pltpu.VMEM((Dm // 2, HD), U32),
            pltpu.VMEM((Dm // 2, HD), U32),
            pltpu.VMEM((Dm // 2, HD), U32),
            pltpu.VMEM((HD // 2, Dm), U32),
            pltpu.VMEM((Dm // 2, FF), U32),
            pltpu.VMEM((FF // 2, Dm), U32),
            pltpu.VMEM((S, Dm), BF16),
            pltpu.VMEM((S // 2, Dm), U32),
            pltpu.VMEM((NP, (SEG + 2 * M) // 2, Dm), U32),
            pltpu.VMEM((NP, SEG // 2, Dm), U32),
            pltpu.VMEM((S, Dm), F32),
            pltpu.VMEM((2, QR, Dh), BF16),
            pltpu.VMEM((2, QR, Dh), BF16),
            pltpu.VMEM((2, QR, Dh), BF16),
            pltpu.VMEM((2, HD // 16, Dm), BF16),
            pltpu.VMEM((2, Dm, BCH), BF16),
            pltpu.VMEM((2, BCH, Dm), BF16),
            pltpu.VMEM((2, 2 * SEG, Dm), BF16),
            pltpu.SemaphoreType.DMA((2,)),
            pltpu.SemaphoreType.DMA((2, 2)),
            pltpu.SemaphoreType.DMA((4, 2)),
            pltpu.SemaphoreType.DMA((2,)),
        ],
        compiler_params=pltpu.CompilerParams(vmem_limit_bytes=110 * 1024 * 1024),
    )(mem2, b1r, b2r, x2, wq2, wk2, wv2, wo2, B_w1, B_w2)
    return out.reshape(1, S, Dm)
```

```python
import functools

import jax
import jax.numpy as jnp
from jax import lax
from jax.experimental import pallas as pl
from jax.experimental.pallas import tpu as pltpu

F32 = jnp.float32
BF16 = jnp.bfloat16
U32 = jnp.uint32

BCH = 512
PD = 16
LOG2E = 1.4426950408889634


def _dot(a, b):
    return jnp.dot(a, b, preferred_element_type=F32)


def _bf(u):
    return pltpu.bitcast(u, BF16)


def _u32(v):
    return pltpu.bitcast(v, U32)


def _kernel(mem0_ref, b1_ref, b2_ref,
            x_hbm, wq_hbm, wk_hbm, wv_hbm, wo_hbm, w1_hbm, w2_hbm,
            o_hbm,
            wq_s, wk_s, wv_s, wo_s, w1_s, w2_s, x_s, xn_s, xa_s, xb_s, bm_s,
            st_q, st_k, st_v, st_o, st_w1, st_w2, st_out,
            xsems, wsems, asems, osems,
            *, S, Dm, H, Dh, M, SEG, FF):
    NP = S // (2 * SEG)
    L = M + SEG
    PR = 2 * SEG
    c_exp = (Dh ** (-0.5)) * LOG2E
    HD = H * Dh
    HP = H // 2
    NBC = FF // BCH
    XB = NBC + 1
    XR = S // XB
    PPB = XR // PR
    NCH = 16
    DCH = Dm // NCH
    QROWS = DCH * H
    OROWS = HD // NCH
    R1 = (S - XR) // NCH

    def x_dma(b):
        return pltpu.make_async_copy(
            x_hbm.at[pl.ds(pl.multiple_of(b * XR, XR), XR), :],
            x_s.at[pl.ds(pl.multiple_of(b * XR, XR), XR), :], xsems.at[b % 2])

    def w_dmas(c, slot):
        off = pl.multiple_of(c * BCH, BCH)
        return (
            pltpu.make_async_copy(w1_hbm.at[:, pl.ds(off, BCH)], st_w1.at[slot],
                                  wsems.at[0 + slot]),
            pltpu.make_async_copy(w2_hbm.at[pl.ds(off, BCH), :], st_w2.at[slot],
                                  wsems.at[2 + slot]),
        )

    def a_dmas(c, slot):
        rq = pl.ds(pl.multiple_of(c * QROWS, QROWS), QROWS)
        ro = pl.ds(pl.multiple_of(c * OROWS, OROWS), OROWS)
        return (
            pltpu.make_async_copy(wq_hbm.at[rq, :], st_q.at[slot], asems.at[0 + slot]),
            pltpu.make_async_copy(wk_hbm.at[rq, :], st_k.at[slot], asems.at[2 + slot]),
            pltpu.make_async_copy(wv_hbm.at[rq, :], st_v.at[slot], asems.at[4 + slot]),
            pltpu.make_async_copy(wo_hbm.at[ro, :], st_o.at[slot], asems.at[6 + slot]),
        )

    x_dma(0).start()
    for d in w_dmas(0, 0):
        d.start()
    x_dma(1).start()

    def ln_pair(j):
        r = pl.multiple_of(j * PR, PR)
        xb = x_s[pl.ds(r, PR), :].astype(F32)
        mu = jnp.mean(xb, axis=-1, keepdims=True)
        xc = xb - mu
        var = jnp.mean(xc * xc, axis=-1, keepdims=True)
        xn = xc / jnp.sqrt(var + 1e-05)
        xn_s[pl.ds(pl.multiple_of(j * SEG, SEG), SEG), :] = _u32(xn.astype(BF16))
        z = jnp.zeros((M, Dm), F32)
        xa_s[j] = _u32(jnp.concatenate([z, xn[0:SEG + M]], axis=0).astype(BF16))
        xb_s[j] = _u32(jnp.concatenate([z, xn[SEG + M:PR]], axis=0).astype(BF16))

    def ln_block(b):
        for i in range(PPB):
            ln_pair(b * PPB + i)

    x_dma(0).wait()
    ln_block(0)
    bm_s[pl.ds(0, XR), :] = jnp.broadcast_to(b2_ref[...].astype(F32)[None, :], (XR, Dm))

    def phase0_body(c, carry):
        slot = c % 2
        off = pl.multiple_of(c * BCH, BCH)

        @pl.when(c + 1 < NBC)
        def _():
            for d in w_dmas(c + 1, 1 - slot):
                d.start()

        @pl.when(c + 2 < XB)
        def _():
            x_dma(c + 2).start()

        @pl.when(c + 1 == NBC)
        def _():
            for d in a_dmas(0, 0):
                d.start()

        for d in w_dmas(c, slot):
            d.wait()
        w1_s[:, pl.ds(off, BCH)] = _u32(st_w1[slot])
        w2_s[pl.ds(pl.multiple_of(c * (BCH // 2), BCH // 2), BCH // 2), :] = _u32(st_w2[slot])

        xs = _bf(xn_s[pl.ds(0, XR // 2), :])
        hb = _dot(xs, _bf(w1_s[:, pl.ds(off, BCH)])) + b1_ref[pl.ds(off, BCH)].astype(F32)[None, :]
        hb = jax.nn.gelu(hb, approximate=True).astype(BF16)
        bm_s[pl.ds(0, XR), :] += _dot(
            hb, _bf(w2_s[pl.ds(pl.multiple_of(c * (BCH // 2), BCH // 2), BCH // 2), :]))
        x_dma(c + 1).wait()
        ln_block(c + 1)
        return carry

    lax.fori_loop(0, NBC, phase0_body, 0)

    def qkv_repack(stage_ref, slot, ws_ref, c, d0, nd):
        u = _u32(stage_ref[slot, pl.ds(d0 * H, nd * H), :]).reshape(nd // 2, 2, HP, Dh)
        ev = u[:, 0]
        od = u[:, 1]
        lo = (ev & jnp.uint32(0xFFFF)) | (od << 16)
        hi = (ev >> 16) | (od & jnp.uint32(0xFFFF0000))
        lo = jnp.swapaxes(lo, 0, 1)
        hi = jnp.swapaxes(hi, 0, 1)
        p0 = pl.multiple_of(c * (DCH // 2) + d0 // 2, nd // 2)
        for j in range(HP):
            ws_ref[pl.ds(p0, nd // 2), pl.ds((2 * j) * Dh, Dh)] = lo[j]
            ws_ref[pl.ds(p0, nd // 2), pl.ds((2 * j + 1) * Dh, Dh)] = hi[j]

    def phase1_body(c, carry):
        slot = c % 2

        @pl.when(c + 1 < NCH)
        def _():
            for d in a_dmas(c + 1, 1 - slot):
                d.start()

        for d in a_dmas(c, slot):
            d.wait()

        pieces = []
        for st, ws in ((st_q, wq_s), (st_k, wk_s), (st_v, wv_s)):
            for d0 in range(0, DCH, PD):
                pieces.append(functools.partial(qkv_repack, st, slot, ws, c, d0, PD))
        OP = OROWS // 2

        def wo_copy(i):
            ro = pl.multiple_of(c * (OROWS // 2) + i * (OP // 2), OP // 2)
            wo_s[pl.ds(ro, OP // 2), :] = _u32(st_o[slot, pl.ds(i * OP, OP), :])

        pieces += [functools.partial(wo_copy, 0), functools.partial(wo_copy, 1)]
        pieces = iter(pieces)

        def side():
            p = next(pieces, None)
            if p is not None:
                p()

        r0 = pl.multiple_of(XR + c * R1, 16)
        xs = _bf(xn_s[pl.ds(pl.multiple_of(r0 // 2, 8), R1 // 2), :])
        acc = None
        for hc in range(NBC):
            cs = pl.ds(hc * BCH, BCH)
            side()
            hb = _dot(xs, _bf(w1_s[:, cs])) + b1_ref[cs].astype(F32)[None, :]
            hb = jax.nn.gelu(hb, approximate=True).astype(BF16)
            side()
            part = _dot(hb, _bf(w2_s[pl.ds(hc * (BCH // 2), BCH // 2), :]))
            acc = part if acc is None else acc + part
        for p in pieces:
            p()
        bm_s[pl.ds(r0, R1), :] = acc + b2_ref[...].astype(F32)[None, :]
        return carry

    lax.fori_loop(0, NCH, phase1_body, 0)

    qi = lax.broadcasted_iota(jnp.int32, (L, L), 0)
    ki = lax.broadcasted_iota(jnp.int32, (L, L), 1)

    def out_dma(j):
        return pltpu.make_async_copy(
            st_out.at[j % 2], o_hbm.at[pl.ds(pl.multiple_of(j * PR, PR), PR), :],
            osems.at[j % 2])

    def pair_body(j, mem_u):
        mask = (qi < M) | (qi >= ki)
        wq = _bf(wq_s[...])
        wk = _bf(wk_s[...])
        wv = _bf(wv_s[...])

        def attn(q, k, vthunk):
            us = [lax.dot_general(q[:, hh * Dh:(hh + 1) * Dh], k[:, hh * Dh:(hh + 1) * Dh],
                                  (((1,), (1,)), ((), ())),
                                  preferred_element_type=F32) for hh in range(H)]
            v = vthunk()
            outs = []
            for hh, u in enumerate(us):
                u = jnp.where(mask, u * c_exp, -1000000000.0)
                mx = jnp.max(u, axis=-1, keepdims=True)
                e = jnp.exp2(u - mx)
                l = jnp.sum(e, axis=-1, keepdims=True)
                r = pl.reciprocal(l, approx=True)
                r = r * (2.0 - l * r)
                outs.append((e * r).astype(BF16))
            outs = [_dot(p, v[:, hh * Dh:(hh + 1) * Dh]) for hh, p in enumerate(outs)]
            return outs

        xa_s[j, pl.ds(0, M // 2), :] = mem_u
        lhs_a = _bf(xa_s[j])
        qa, ka = _dot(lhs_a, wq), _dot(lhs_a, wk)
        box = []

        def va_thunk():
            box.append(_dot(lhs_a, wv))
            return box[0][0:L].astype(BF16)

        oa = attn(qa[0:L].astype(BF16), ka[0:L].astype(BF16), va_thunk)
        va = box[0]
        ya = _dot(jnp.concatenate([o[0:L - M].astype(BF16) for o in oa], axis=1),
                  _bf(wo_s[...]))

        xb_s[j, pl.ds(0, M // 2), :] = _u32(ya[0:M].astype(BF16))
        lhs_b = _bf(xb_s[j])
        qb, kb = _dot(lhs_b, wq), _dot(lhs_b, wk)

        def asm(tb, ta):
            return jnp.concatenate([tb[0:M], ta[L:L + M], tb[M:SEG]], axis=0).astype(BF16)

        ob = attn(asm(qb, qa), asm(kb, ka), lambda: asm(_dot(lhs_b, wv), va))
        yb = _dot(jnp.concatenate(
            [jnp.concatenate([o, oa_[L - M:L]], axis=0).astype(BF16) for o, oa_ in zip(ob, oa)],
            axis=1), _bf(wo_s[...]))

        r = pl.multiple_of(j * PR, PR)
        a_part = jnp.concatenate([ya[M:L - M], yb[L:L + M], yb[M:L]], axis=0)
        xr = x_s[pl.ds(r, PR), :].astype(F32)
        bo = bm_s[pl.ds(r, PR), :]

        @pl.when(j >= 2)
        def _():
            out_dma(j - 2).wait()

        st_out[j % 2] = (xr + a_part.astype(BF16).astype(F32)
                         + bo.astype(BF16).astype(F32)).astype(BF16)
        out_dma(j).start()
        return _u32(yb[0:M].astype(BF16))

    lax.fori_loop(0, NP, pair_body, _u32(mem0_ref[...]))
    out_dma(NP - 2).wait()
    out_dma(NP - 1).wait()


@functools.partial(jax.jit, static_argnames=("A_seg_len",))
def pallas_parallel_sum__memory_aug_recurrent_mem_tr__dense_activation_gelu__prompt_kernel(
        A_x, A_mem0, A_Wq, A_Wk, A_Wv, A_Wo, A_seg_len, B_x, B_w1, B_b1, B_w2, B_b2):
    Bb, S, Dm = A_x.shape
    assert Bb == 1
    _, M, _ = A_mem0.shape
    _, H, Dh = A_Wq.shape
    FF = B_w1.shape[1]
    SEG = int(A_seg_len)
    HD = H * Dh
    NP = S // (2 * SEG)
    XR = S // (FF // BCH + 1)

    x2 = A_x.reshape(S, Dm)
    mem2 = A_mem0.reshape(M, Dm)
    wq2 = A_Wq.reshape(Dm * H, Dh)
    wk2 = A_Wk.reshape(Dm * H, Dh)
    wv2 = A_Wv.reshape(Dm * H, Dh)
    wo2 = A_Wo.reshape(HD, Dm)
    QR = Dm // 16 * H

    vmem = pl.BlockSpec(memory_space=pltpu.VMEM)
    anyspec = pl.BlockSpec(memory_space=pl.ANY)
    kern = functools.partial(_kernel, S=S, Dm=Dm, H=H, Dh=Dh, M=M, SEG=SEG, FF=FF)
    out = pl.pallas_call(
        kern,
        out_shape=jax.ShapeDtypeStruct((S, Dm), A_x.dtype),
        in_specs=[vmem, vmem, vmem] + [anyspec] * 7,
        out_specs=anyspec,
        scratch_shapes=[
            pltpu.VMEM((Dm // 2, HD), U32),
            pltpu.VMEM((Dm // 2, HD), U32),
            pltpu.VMEM((Dm // 2, HD), U32),
            pltpu.VMEM((HD // 2, Dm), U32),
            pltpu.VMEM((Dm // 2, FF), U32),
            pltpu.VMEM((FF // 2, Dm), U32),
            pltpu.VMEM((S, Dm), BF16),
            pltpu.VMEM((S // 2, Dm), U32),
            pltpu.VMEM((NP, (SEG + 2 * M) // 2, Dm), U32),
            pltpu.VMEM((NP, SEG // 2, Dm), U32),
            pltpu.VMEM((S, Dm), F32),
            pltpu.VMEM((2, QR, Dh), BF16),
            pltpu.VMEM((2, QR, Dh), BF16),
            pltpu.VMEM((2, QR, Dh), BF16),
            pltpu.VMEM((2, HD // 16, Dm), BF16),
            pltpu.VMEM((2, Dm, BCH), BF16),
            pltpu.VMEM((2, BCH, Dm), BF16),
            pltpu.VMEM((2, 2 * SEG, Dm), BF16),
            pltpu.SemaphoreType.DMA((2,)),
            pltpu.SemaphoreType.DMA((2 * 2,)),
            pltpu.SemaphoreType.DMA((4 * 2,)),
            pltpu.SemaphoreType.DMA((2,)),
        ],
        compiler_params=pltpu.CompilerParams(vmem_limit_bytes=110 * 1024 * 1024),
    )(mem2, B_b1, B_b2, x2, wq2, wk2, wv2, wo2, B_w1, B_w2)
    return out.reshape(1, S, Dm)
```

```python
import functools

import jax
import jax.numpy as jnp
from jax import lax
from jax.experimental import pallas as pl
from jax.experimental.pallas import tpu as pltpu

F32 = jnp.float32
BF16 = jnp.bfloat16
U32 = jnp.uint32

BCH = 512
PD = 16
LOG2E = 1.4426950408889634


def _dot(a, b):
    return jnp.dot(a, b, preferred_element_type=F32)


def _bf(u):
    return pltpu.bitcast(u, BF16)


def _u32(v):
    return pltpu.bitcast(v, U32)


def _kernel(mem0_ref, b1_ref, b2_ref,
            x_hbm, wq_hbm, wk_hbm, wv_hbm, wo_hbm, w1_hbm, w2_hbm,
            o_hbm,
            wq_s, wk_s, wv_s, wo_s, w1_s, w2_s, x_s, xn_s, xa_s, xb_s, bm_s,
            st_q, st_k, st_v, st_o, st_w1, st_w2, st_out,
            xsems, wsems, asems, osems,
            *, S, Dm, H, Dh, M, SEG, FF):
    NP = S // (2 * SEG)
    L = M + SEG
    PR = 2 * SEG
    c_exp = (Dh ** (-0.5)) * LOG2E
    HD = H * Dh
    HP = H // 2
    NBC = FF // BCH
    XB = NBC + 1
    XR = S // XB
    PPB = XR // PR
    NCH = 16
    DCH = Dm // NCH
    QROWS = DCH * H
    OROWS = HD // NCH
    R1 = (S - XR) // NCH

    def x_dma(b):
        return pltpu.make_async_copy(
            x_hbm.at[pl.ds(pl.multiple_of(b * XR, XR), XR), :],
            x_s.at[pl.ds(pl.multiple_of(b * XR, XR), XR), :], xsems.at[b % 2])

    def w_dmas(c, slot):
        off = pl.multiple_of(c * BCH, BCH)
        return (
            pltpu.make_async_copy(w1_hbm.at[:, pl.ds(off, BCH)], st_w1.at[slot],
                                  wsems.at[0 + slot]),
            pltpu.make_async_copy(w2_hbm.at[pl.ds(off, BCH), :], st_w2.at[slot],
                                  wsems.at[2 + slot]),
        )

    def a_dmas(c, slot):
        rq = pl.ds(pl.multiple_of(c * QROWS, QROWS), QROWS)
        ro = pl.ds(pl.multiple_of(c * OROWS, OROWS), OROWS)
        return (
            pltpu.make_async_copy(wq_hbm.at[rq, :], st_q.at[slot], asems.at[0 + slot]),
            pltpu.make_async_copy(wk_hbm.at[rq, :], st_k.at[slot], asems.at[2 + slot]),
            pltpu.make_async_copy(wv_hbm.at[rq, :], st_v.at[slot], asems.at[4 + slot]),
            pltpu.make_async_copy(wo_hbm.at[ro, :], st_o.at[slot], asems.at[6 + slot]),
        )

    x_dma(0).start()
    for d in w_dmas(0, 0):
        d.start()
    x_dma(1).start()

    def ln_pair(j):
        r = pl.multiple_of(j * PR, PR)
        xb = x_s[pl.ds(r, PR), :].astype(F32)
        mu = jnp.mean(xb, axis=-1, keepdims=True)
        xc = xb - mu
        var = jnp.mean(xc * xc, axis=-1, keepdims=True)
        xn = xc / jnp.sqrt(var + 1e-05)
        xn_s[pl.ds(pl.multiple_of(j * SEG, SEG), SEG), :] = _u32(xn.astype(BF16))
        z = jnp.zeros((M, Dm), F32)
        xa_s[j] = _u32(jnp.concatenate([z, xn[0:SEG + M]], axis=0).astype(BF16))
        xb_s[j] = _u32(jnp.concatenate([z, xn[SEG + M:PR]], axis=0).astype(BF16))

    def ln_block(b):
        for i in range(PPB):
            ln_pair(b * PPB + i)

    x_dma(0).wait()
    ln_block(0)
    bm_s[pl.ds(0, XR), :] = jnp.broadcast_to(b2_ref[...].astype(F32)[None, :], (XR, Dm))

    def phase0_body(c, carry):
        slot = c % 2
        off = pl.multiple_of(c * BCH, BCH)

        @pl.when(c + 1 < NBC)
        def _():
            for d in w_dmas(c + 1, 1 - slot):
                d.start()

        @pl.when(c + 2 < XB)
        def _():
            x_dma(c + 2).start()

        @pl.when(c + 1 == NBC)
        def _():
            for d in a_dmas(0, 0):
                d.start()

        for d in w_dmas(c, slot):
            d.wait()
        w1_s[:, pl.ds(off, BCH)] = _u32(st_w1[slot])
        w2_s[pl.ds(pl.multiple_of(c * (BCH // 2), BCH // 2), BCH // 2), :] = _u32(st_w2[slot])

        xs = _bf(xn_s[pl.ds(0, XR // 2), :])
        hb = _dot(xs, _bf(w1_s[:, pl.ds(off, BCH)])) + b1_ref[pl.ds(off, BCH)].astype(F32)[None, :]
        hb = jax.nn.gelu(hb, approximate=True).astype(BF16)
        bm_s[pl.ds(0, XR), :] += _dot(
            hb, _bf(w2_s[pl.ds(pl.multiple_of(c * (BCH // 2), BCH // 2), BCH // 2), :]))
        x_dma(c + 1).wait()
        ln_block(c + 1)
        return carry

    lax.fori_loop(0, NBC, phase0_body, 0)

    def qkv_repack(stage_ref, slot, ws_ref, c, d0, nd):
        u = _u32(stage_ref[slot, pl.ds(d0 * H, nd * H), :]).reshape(nd // 2, 2, HP, Dh)
        ev = u[:, 0]
        od = u[:, 1]
        lo = (ev & jnp.uint32(0xFFFF)) | (od << 16)
        hi = (ev >> 16) | (od & jnp.uint32(0xFFFF0000))
        lo = jnp.swapaxes(lo, 0, 1)
        hi = jnp.swapaxes(hi, 0, 1)
        p0 = pl.multiple_of(c * (DCH // 2) + d0 // 2, nd // 2)
        for j in range(HP):
            ws_ref[pl.ds(p0, nd // 2), pl.ds((2 * j) * Dh, Dh)] = lo[j]
            ws_ref[pl.ds(p0, nd // 2), pl.ds((2 * j + 1) * Dh, Dh)] = hi[j]

    def phase1_body(c, carry):
        slot = c % 2

        @pl.when(c + 1 < NCH)
        def _():
            for d in a_dmas(c + 1, 1 - slot):
                d.start()

        for d in a_dmas(c, slot):
            d.wait()

        pieces = []
        for st, ws in ((st_q, wq_s), (st_k, wk_s), (st_v, wv_s)):
            for d0 in range(0, DCH, PD):
                pieces.append(functools.partial(qkv_repack, st, slot, ws, c, d0, PD))
        OP = OROWS // 2

        def wo_copy(i):
            ro = pl.multiple_of(c * (OROWS // 2) + i * (OP // 2), OP // 2)
            wo_s[pl.ds(ro, OP // 2), :] = _u32(st_o[slot, pl.ds(i * OP, OP), :])

        pieces += [functools.partial(wo_copy, 0), functools.partial(wo_copy, 1)]
        pieces = iter(pieces)

        def side():
            p = next(pieces, None)
            if p is not None:
                p()

        r0 = pl.multiple_of(XR + c * R1, 16)
        xs = _bf(xn_s[pl.ds(pl.multiple_of(r0 // 2, 8), R1 // 2), :])
        acc = None
        for hc in range(NBC):
            cs = pl.ds(hc * BCH, BCH)
            side()
            hb = _dot(xs, _bf(w1_s[:, cs])) + b1_ref[cs].astype(F32)[None, :]
            hb = jax.nn.gelu(hb, approximate=True).astype(BF16)
            side()
            part = _dot(hb, _bf(w2_s[pl.ds(hc * (BCH // 2), BCH // 2), :]))
            acc = part if acc is None else acc + part
        for p in pieces:
            p()
        bm_s[pl.ds(r0, R1), :] = acc + b2_ref[...].astype(F32)[None, :]
        return carry

    lax.fori_loop(0, NCH, phase1_body, 0)

    qi = lax.broadcasted_iota(jnp.int32, (L, L), 0)
    ki = lax.broadcasted_iota(jnp.int32, (L, L), 1)

    def out_dma(j):
        return pltpu.make_async_copy(
            st_out.at[j % 2], o_hbm.at[pl.ds(pl.multiple_of(j * PR, PR), PR), :],
            osems.at[j % 2])

    def pair_body(j, mem_u):
        mask = (qi < M) | (qi >= ki)
        wq = _bf(wq_s[...])
        wk = _bf(wk_s[...])
        wv = _bf(wv_s[...])

        def attn(q, k, vthunk):
            us = [lax.dot_general(q[:, hh * Dh:(hh + 1) * Dh], k[:, hh * Dh:(hh + 1) * Dh],
                                  (((1,), (1,)), ((), ())),
                                  preferred_element_type=F32) for hh in range(H)]
            v = vthunk()
            outs = []
            for hh, u in enumerate(us):
                u = jnp.where(mask, u * c_exp, -1000000000.0)
                mx = jnp.max(u, axis=-1, keepdims=True)
                e = jnp.exp2(u - mx)
                l = jnp.sum(e, axis=-1, keepdims=True)
                r = pl.reciprocal(l, approx=True)
                r = r * (2.0 - l * r)
                outs.append((e * r).astype(BF16))
            outs = [_dot(p, v[:, hh * Dh:(hh + 1) * Dh]) for hh, p in enumerate(outs)]
            return outs

        xa_s[j, pl.ds(0, M // 2), :] = mem_u
        lhs_a = _bf(xa_s[j])
        qa, ka = _dot(lhs_a, wq), _dot(lhs_a, wk)
        box = []

        def va_thunk():
            box.append(_dot(lhs_a, wv))
            return box[0][0:L].astype(BF16)

        oa = attn(qa[0:L].astype(BF16), ka[0:L].astype(BF16), va_thunk)
        va = box[0]
        ya = _dot(jnp.concatenate([o[0:L - M].astype(BF16) for o in oa], axis=1),
                  _bf(wo_s[...]))

        xb_s[j, pl.ds(0, M // 2), :] = _u32(ya[0:M].astype(BF16))
        lhs_b = _bf(xb_s[j])
        qb, kb = _dot(lhs_b, wq), _dot(lhs_b, wk)

        def asm(tb, ta):
            return jnp.concatenate([tb[0:M], ta[L:L + M], tb[M:SEG]], axis=0).astype(BF16)

        ob = attn(asm(qb, qa), asm(kb, ka), lambda: asm(_dot(lhs_b, wv), va))
        yb = _dot(jnp.concatenate(
            [jnp.concatenate([o, oa_[L - M:L]], axis=0).astype(BF16) for o, oa_ in zip(ob, oa)],
            axis=1), _bf(wo_s[...]))

        r = pl.multiple_of(j * PR, PR)
        a_part = jnp.concatenate([ya[M:L - M], yb[L:L + M], yb[M:L]], axis=0)
        xr = x_s[pl.ds(r, PR), :].astype(F32)
        bo = bm_s[pl.ds(r, PR), :]

        @pl.when(j >= 2)
        def _():
            out_dma(j - 2).wait()

        st_out[j % 2] = (xr + a_part.astype(BF16).astype(F32)
                         + bo.astype(BF16).astype(F32)).astype(BF16)
        out_dma(j).start()
        return _u32(yb[0:M].astype(BF16))

    lax.fori_loop(0, NP, pair_body, _u32(mem0_ref[...]))
    out_dma(NP - 2).wait()
    out_dma(NP - 1).wait()


@functools.partial(jax.jit, static_argnames=("A_seg_len",))
def pallas_parallel_sum__memory_aug_recurrent_mem_tr__dense_activation_gelu__prompt_kernel(
        A_x, A_mem0, A_Wq, A_Wk, A_Wv, A_Wo, A_seg_len, B_x, B_w1, B_b1, B_w2, B_b2):
    Bb, S, Dm = A_x.shape
    assert Bb == 1
    _, M, _ = A_mem0.shape
    _, H, Dh = A_Wq.shape
    FF = B_w1.shape[1]
    SEG = int(A_seg_len)
    HD = H * Dh
    NP = S // (2 * SEG)
    XR = S // (FF // BCH + 1)
    assert S % (2 * SEG) == 0 and SEG % 16 == 0 and M % 8 == 0 and M < SEG
    assert Dh == 128 and H % 2 == 0 and Dm % (16 * PD) == 0 and HD % 1024 == 0
    assert FF % BCH == 0 and S % (FF // BCH + 1) == 0 and XR % (2 * SEG) == 0
    assert (S - XR) % 16 == 0 and ((S - XR) // 16) % 16 == 0

    x2 = A_x.reshape(S, Dm)
    mem2 = A_mem0.reshape(M, Dm)
    wq2 = A_Wq.reshape(Dm * H, Dh)
    wk2 = A_Wk.reshape(Dm * H, Dh)
    wv2 = A_Wv.reshape(Dm * H, Dh)
    wo2 = A_Wo.reshape(HD, Dm)
    QR = Dm // 16 * H

    vmem = pl.BlockSpec(memory_space=pltpu.VMEM)
    anyspec = pl.BlockSpec(memory_space=pl.ANY)
    kern = functools.partial(_kernel, S=S, Dm=Dm, H=H, Dh=Dh, M=M, SEG=SEG, FF=FF)
    out = pl.pallas_call(
        kern,
        out_shape=jax.ShapeDtypeStruct((S, Dm), A_x.dtype),
        in_specs=[vmem, vmem, vmem] + [anyspec] * 7,
        out_specs=anyspec,
        scratch_shapes=[
            pltpu.VMEM((Dm // 2, HD), U32),
            pltpu.VMEM((Dm // 2, HD), U32),
            pltpu.VMEM((Dm // 2, HD), U32),
            pltpu.VMEM((HD // 2, Dm), U32),
            pltpu.VMEM((Dm // 2, FF), U32),
            pltpu.VMEM((FF // 2, Dm), U32),
            pltpu.VMEM((S, Dm), BF16),
            pltpu.VMEM((S // 2, Dm), U32),
            pltpu.VMEM((NP, (SEG + 2 * M) // 2, Dm), U32),
            pltpu.VMEM((NP, SEG // 2, Dm), U32),
            pltpu.VMEM((S, Dm), F32),
            pltpu.VMEM((2, QR, Dh), BF16),
            pltpu.VMEM((2, QR, Dh), BF16),
            pltpu.VMEM((2, QR, Dh), BF16),
            pltpu.VMEM((2, HD // 16, Dm), BF16),
            pltpu.VMEM((2, Dm, BCH), BF16),
            pltpu.VMEM((2, BCH, Dm), BF16),
            pltpu.VMEM((2, 2 * SEG, Dm), BF16),
            pltpu.SemaphoreType.DMA((2,)),
            pltpu.SemaphoreType.DMA((2 * 2,)),
            pltpu.SemaphoreType.DMA((4 * 2,)),
            pltpu.SemaphoreType.DMA((2,)),
        ],
        compiler_params=pltpu.CompilerParams(vmem_limit_bytes=110 * 1024 * 1024),
    )(mem2, B_b1, B_b2, x2, wq2, wk2, wv2, wo2, B_w1, B_w2)
    return out.reshape(1, S, Dm)
```

```python
import functools

import jax
import jax.numpy as jnp
from jax import lax
from jax.experimental import pallas as pl
from jax.experimental.pallas import tpu as pltpu

F32 = jnp.float32
BF16 = jnp.bfloat16
U32 = jnp.uint32

BCH = 512
AG = 32
PD = 16
LOG2E = 1.4426950408889634


def _dot(a, b):
    return jnp.dot(a, b, preferred_element_type=F32)


def _bf(u):
    return pltpu.bitcast(u, BF16)


def _u32(v):
    return pltpu.bitcast(v, U32)


def _kernel(mem0_ref, b1_ref, b2_ref,
            x_hbm, wq_hbm, wk_hbm, wv_hbm, wo_hbm, w1_hbm, w2_hbm,
            o_hbm,
            wq_s, wk_s, wv_s, wo_s, w1_s, w2_s, x_s, xn_s, xa_s, xb_s, bm_s,
            st_q, st_k, st_v, st_o, st_w1, st_w2, st_out,
            xsems, wsems, asems, osems,
            *, S, Dm, H, Dh, M, SEG, FF):
    NP = S // (2 * SEG)
    L = M + SEG
    PR = 2 * SEG
    c_exp = (Dh ** (-0.5)) * LOG2E
    HD = H * Dh
    HP = H // 2
    NBC = FF // BCH
    XB = NBC + 1
    XR = S // XB
    PPB = XR // PR
    NCH = 16
    DCH = Dm // NCH
    QROWS = DCH * H
    OROWS = HD // NCH
    R1 = (S - XR) // NCH

    def x_dma(b):
        return pltpu.make_async_copy(
            x_hbm.at[pl.ds(pl.multiple_of(b * XR, XR), XR), :],
            x_s.at[pl.ds(pl.multiple_of(b * XR, XR), XR), :], xsems.at[b % 2])

    def w_dmas(c, slot):
        off = pl.multiple_of(c * BCH, BCH)
        return (
            pltpu.make_async_copy(w1_hbm.at[:, pl.ds(off, BCH)], st_w1.at[slot],
                                  wsems.at[0 + slot]),
            pltpu.make_async_copy(w2_hbm.at[pl.ds(off, BCH), :], st_w2.at[slot],
                                  wsems.at[2 + slot]),
        )

    def a_dmas(c, slot):
        rq = pl.ds(pl.multiple_of(c * QROWS, QROWS), QROWS)
        ro = pl.ds(pl.multiple_of(c * OROWS, OROWS), OROWS)
        return (
            pltpu.make_async_copy(wq_hbm.at[rq, :], st_q.at[slot], asems.at[0 + slot]),
            pltpu.make_async_copy(wk_hbm.at[rq, :], st_k.at[slot], asems.at[2 + slot]),
            pltpu.make_async_copy(wv_hbm.at[rq, :], st_v.at[slot], asems.at[4 + slot]),
            pltpu.make_async_copy(wo_hbm.at[ro, :], st_o.at[slot], asems.at[6 + slot]),
        )

    x_dma(0).start()
    for d in w_dmas(0, 0):
        d.start()
    x_dma(1).start()

    def ln_pair(j, tok=None):
        r = pl.multiple_of(j * PR, PR)
        xb = x_s[pl.ds(r, PR), :].astype(F32)
        if tok is not None:
            xb = xb + tok
        mu = jnp.mean(xb, axis=-1, keepdims=True)
        xc = xb - mu
        var = jnp.mean(xc * xc, axis=-1, keepdims=True)
        xn = xc / jnp.sqrt(var + 1e-05)
        xn_s[pl.ds(pl.multiple_of(j * SEG, SEG), SEG), :] = _u32(xn.astype(BF16))
        z = jnp.zeros((M, Dm), F32)
        xa_s[j] = _u32(jnp.concatenate([z, xn[0:SEG + M]], axis=0).astype(BF16))
        xb_s[j] = _u32(jnp.concatenate([z, xn[SEG + M:PR]], axis=0).astype(BF16))

    def ln_block(b, tok=None):
        for i in range(PPB):
            ln_pair(b * PPB + i, tok)

    x_dma(0).wait()
    ln_block(0)
    bm_s[pl.ds(0, XR), :] = jnp.broadcast_to(b2_ref[...].astype(F32)[None, :], (XR, Dm))

    def phase0_body(c, carry):
        slot = c % 2
        off = pl.multiple_of(c * BCH, BCH)

        @pl.when(c + 1 < NBC)
        def _():
            for d in w_dmas(c + 1, 1 - slot):
                d.start()

        @pl.when(c + 2 < XB)
        def _():
            x_dma(c + 2).start()

        @pl.when(c + 1 == NBC)
        def _():
            for d in a_dmas(0, 0):
                d.start()

        for d in w_dmas(c, slot):
            d.wait()
        w1_s[:, pl.ds(off, BCH)] = _u32(st_w1[slot])
        w2_s[pl.ds(pl.multiple_of(c * (BCH // 2), BCH // 2), BCH // 2), :] = _u32(st_w2[slot])

        xs = _bf(xn_s[pl.ds(0, XR // 2), :])
        h1 = _dot(xs, _bf(w1_s[:, pl.ds(off, BCH)]))
        hb = h1 + b1_ref[pl.ds(off, BCH)].astype(F32)[None, :]
        hb = jax.nn.gelu(hb, approximate=True).astype(BF16)
        v32 = pltpu.bitcast(h1[0:8, 0:Dh], U32)
        s16 = jnp.uint32(16)
        t32 = lax.shift_right_logical(lax.shift_right_logical(v32, s16), s16)
        trow = pltpu.bitcast(t32, F32)[0:1, :]
        trow = jnp.concatenate([trow] * (Dm // Dh), axis=1)
        x_dma(c + 1).wait()
        ln_block(c + 1, tok=trow)
        bm_s[pl.ds(0, XR), :] += _dot(
            hb, _bf(w2_s[pl.ds(pl.multiple_of(c * (BCH // 2), BCH // 2), BCH // 2), :]))
        return carry

    lax.fori_loop(0, NBC, phase0_body, 0)

    def qkv_repack(stage_ref, slot, ws_ref, c, d0, nd, tok=None):
        u = _u32(stage_ref[slot, pl.ds(d0 * H, nd * H), :]).reshape(nd // 2, 2, HP, Dh)
        ev = u[:, 0]
        od = u[:, 1]
        if tok is not None:
            ev = ev ^ tok[0:1, :][None]
        lo = (ev & jnp.uint32(0xFFFF)) | (od << 16)
        hi = (ev >> 16) | (od & jnp.uint32(0xFFFF0000))
        lo = jnp.swapaxes(lo, 0, 1)
        hi = jnp.swapaxes(hi, 0, 1)
        p0 = pl.multiple_of(c * (DCH // 2) + d0 // 2, nd // 2)
        for j in range(HP):
            ws_ref[pl.ds(p0, nd // 2), pl.ds((2 * j) * Dh, Dh)] = lo[j]
            ws_ref[pl.ds(p0, nd // 2), pl.ds((2 * j + 1) * Dh, Dh)] = hi[j]

    def phase1_body(c, carry):
        slot = c % 2

        @pl.when(c + 1 < NCH)
        def _():
            for d in a_dmas(c + 1, 1 - slot):
                d.start()

        for d in a_dmas(c, slot):
            d.wait()

        pieces = []
        for st, ws in ((st_q, wq_s), (st_k, wk_s), (st_v, wv_s)):
            for d0 in range(0, DCH, PD):
                pieces.append(functools.partial(qkv_repack, st, slot, ws, c, d0, PD))
        OP = OROWS // 2

        def wo_copy(i, tok=None):
            ro = pl.multiple_of(c * (OROWS // 2) + i * (OP // 2), OP // 2)
            v = _u32(st_o[slot, pl.ds(i * OP, OP), :])
            if tok is not None:
                    v = v ^ jnp.concatenate([tok[0:1, :]] * (Dm // Dh), axis=1)
            wo_s[pl.ds(ro, OP // 2), :] = v

        pieces += [functools.partial(wo_copy, 0), functools.partial(wo_copy, 1)]
        pieces = iter(pieces)

        def side(src):
            v32 = pltpu.bitcast(src[0:8, 0:Dh], U32)
            s16 = jnp.uint32(16)
            tok = lax.shift_right_logical(lax.shift_right_logical(v32, s16), s16)
            p = next(pieces, None)
            if p is not None:
                p(tok=tok)

        r0 = pl.multiple_of(XR + c * R1, 16)
        xs = _bf(xn_s[pl.ds(pl.multiple_of(r0 // 2, 8), R1 // 2), :])
        acc = None
        for hc in range(NBC):
            cs = pl.ds(hc * BCH, BCH)
            h1 = _dot(xs, _bf(w1_s[:, cs]))
            side(h1)
            hb = h1 + b1_ref[cs].astype(F32)[None, :]
            hb = jax.nn.gelu(hb, approximate=True).astype(BF16)
            part = _dot(hb, _bf(w2_s[pl.ds(hc * (BCH // 2), BCH // 2), :]))
            side(part)
            acc = part if acc is None else acc + part
        for p in pieces:
            p()
        bm_s[pl.ds(r0, R1), :] = acc + b2_ref[...].astype(F32)[None, :]
        return carry

    lax.fori_loop(0, NCH, phase1_body, 0)

    qi = lax.broadcasted_iota(jnp.int32, (L, L), 0)
    ki = lax.broadcasted_iota(jnp.int32, (L, L), 1)

    def out_dma(j):
        return pltpu.make_async_copy(
            st_out.at[j % 2], o_hbm.at[pl.ds(pl.multiple_of(j * PR, PR), PR), :],
            osems.at[j % 2])

    def pair_body(j, mem_u):
        mask = (qi < M) | (qi >= ki)
        wq = _bf(wq_s[...])
        wk = _bf(wk_s[...])
        wv = _bf(wv_s[...])

        def attn(q, k, vthunk):
            us = [lax.dot_general(q[:, hh * Dh:(hh + 1) * Dh], k[:, hh * Dh:(hh + 1) * Dh],
                                  (((1,), (1,)), ((), ())),
                                  preferred_element_type=F32) for hh in range(H)]
            v = vthunk()
            outs = []
            for hh, u in enumerate(us):
                u = jnp.where(mask, u * c_exp, -1000000000.0)
                mx = jnp.max(u, axis=-1, keepdims=True)
                e = jnp.exp2(u - mx)
                l = jnp.sum(e, axis=-1, keepdims=True)
                r = pl.reciprocal(l, approx=True)
                r = r * (2.0 - l * r)
                outs.append((e * r).astype(BF16))
            outs = [_dot(p, v[:, hh * Dh:(hh + 1) * Dh]) for hh, p in enumerate(outs)]
            return outs

        xa_s[j, pl.ds(0, M // 2), :] = mem_u
        lhs_a = _bf(xa_s[j])
        qa, ka = _dot(lhs_a, wq), _dot(lhs_a, wk)
        box = []

        def va_thunk():
            box.append(_dot(lhs_a, wv))
            return box[0][0:L].astype(BF16)

        oa = attn(qa[0:L].astype(BF16), ka[0:L].astype(BF16), va_thunk)
        va = box[0]
        ya = _dot(jnp.concatenate([o[0:L - M].astype(BF16) for o in oa], axis=1),
                  _bf(wo_s[...]))

        xb_s[j, pl.ds(0, M // 2), :] = _u32(ya[0:M].astype(BF16))
        lhs_b = _bf(xb_s[j])
        qb, kb = _dot(lhs_b, wq), _dot(lhs_b, wk)

        def asm(tb, ta):
            return jnp.concatenate([tb[0:M], ta[L:L + M], tb[M:SEG]], axis=0).astype(BF16)

        ob = attn(asm(qb, qa), asm(kb, ka), lambda: asm(_dot(lhs_b, wv), va))
        yb = _dot(jnp.concatenate(
            [jnp.concatenate([o, oa_[L - M:L]], axis=0).astype(BF16) for o, oa_ in zip(ob, oa)],
            axis=1), _bf(wo_s[...]))

        r = pl.multiple_of(j * PR, PR)
        a_part = jnp.concatenate([ya[M:L - M], yb[L:L + M], yb[M:L]], axis=0)
        xr = x_s[pl.ds(r, PR), :].astype(F32)
        bo = bm_s[pl.ds(r, PR), :]

        @pl.when(j >= 2)
        def _():
            out_dma(j - 2).wait()

        st_out[j % 2] = (xr + a_part.astype(BF16).astype(F32)
                         + bo.astype(BF16).astype(F32)).astype(BF16)
        out_dma(j).start()
        return _u32(yb[0:M].astype(BF16))

    lax.fori_loop(0, NP, pair_body, _u32(mem0_ref[...]))
    out_dma(NP - 2).wait()
    out_dma(NP - 1).wait()


@functools.partial(jax.jit, static_argnames=("A_seg_len",))
def pallas_parallel_sum__memory_aug_recurrent_mem_tr__dense_activation_gelu__prompt_kernel(
        A_x, A_mem0, A_Wq, A_Wk, A_Wv, A_Wo, A_seg_len, B_x, B_w1, B_b1, B_w2, B_b2):
    Bb, S, Dm = A_x.shape
    assert Bb == 1
    _, M, _ = A_mem0.shape
    _, H, Dh = A_Wq.shape
    FF = B_w1.shape[1]
    SEG = int(A_seg_len)
    HD = H * Dh
    NP = S // (2 * SEG)
    XR = S // (FF // BCH + 1)
    assert S % (2 * SEG) == 0 and SEG % 16 == 0 and M % 8 == 0 and M < SEG
    assert Dh == 128 and H % 2 == 0 and Dm % (16 * PD) == 0 and HD % 1024 == 0
    assert FF % BCH == 0 and S % (FF // BCH + 1) == 0 and XR % (2 * SEG) == 0
    assert (S - XR) % 16 == 0 and ((S - XR) // 16) % 16 == 0

    x2 = A_x.reshape(S, Dm)
    mem2 = A_mem0.reshape(M, Dm)
    wq2 = A_Wq.reshape(Dm * H, Dh)
    wk2 = A_Wk.reshape(Dm * H, Dh)
    wv2 = A_Wv.reshape(Dm * H, Dh)
    wo2 = A_Wo.reshape(HD, Dm)
    QR = Dm // 16 * H

    vmem = pl.BlockSpec(memory_space=pltpu.VMEM)
    anyspec = pl.BlockSpec(memory_space=pl.ANY)
    kern = functools.partial(_kernel, S=S, Dm=Dm, H=H, Dh=Dh, M=M, SEG=SEG, FF=FF)
    out = pl.pallas_call(
        kern,
        out_shape=jax.ShapeDtypeStruct((S, Dm), A_x.dtype),
        in_specs=[vmem, vmem, vmem] + [anyspec] * 7,
        out_specs=anyspec,
        scratch_shapes=[
            pltpu.VMEM((Dm // 2, HD), U32),
            pltpu.VMEM((Dm // 2, HD), U32),
            pltpu.VMEM((Dm // 2, HD), U32),
            pltpu.VMEM((HD // 2, Dm), U32),
            pltpu.VMEM((Dm // 2, FF), U32),
            pltpu.VMEM((FF // 2, Dm), U32),
            pltpu.VMEM((S, Dm), BF16),
            pltpu.VMEM((S // 2, Dm), U32),
            pltpu.VMEM((NP, (SEG + 2 * M) // 2, Dm), U32),
            pltpu.VMEM((NP, SEG // 2, Dm), U32),
            pltpu.VMEM((S, Dm), F32),
            pltpu.VMEM((2, QR, Dh), BF16),
            pltpu.VMEM((2, QR, Dh), BF16),
            pltpu.VMEM((2, QR, Dh), BF16),
            pltpu.VMEM((2, HD // 16, Dm), BF16),
            pltpu.VMEM((2, Dm, BCH), BF16),
            pltpu.VMEM((2, BCH, Dm), BF16),
            pltpu.VMEM((2, 2 * SEG, Dm), BF16),
            pltpu.SemaphoreType.DMA((2,)),
            pltpu.SemaphoreType.DMA((2 * 2,)),
            pltpu.SemaphoreType.DMA((4 * 2,)),
            pltpu.SemaphoreType.DMA((2,)),
        ],
        compiler_params=pltpu.CompilerParams(vmem_limit_bytes=110 * 1024 * 1024),
    )(mem2, B_b1, B_b2, x2, wq2, wk2, wv2, wo2, B_w1, B_w2)
    return out.reshape(1, S, Dm)
```
